```python
import jax
import jax.numpy as jnp

def _softmax(x, axis=-1):
    return jax.nn.softmax(x, axis=axis)
def _gelu(x):
    return jax.nn.gelu(x, approximate=True)
def _silu(x):
    return jax.nn.silu(x)
def _sigmoid(x):
    return jax.nn.sigmoid(x)
def _layernorm(x, axis=-1, eps=1e-5):
    m = jnp.mean(x, axis=axis, keepdims=True)
    v = jnp.var(x, axis=axis, keepdims=True)
    return (x - m) / jnp.sqrt(v + eps)
def _scatter_add(tgt, idx, src, axis=0):
    return tgt.at[idx].add(src)
def _segment_sum(src, seg, n):
    return jax.ops.segment_sum(src, seg, n)
class _Rng:
    def __init__(self, key):
        self._k = key
    def _next(self):
        self._k, sub = jax.random.split(self._k)
        return sub
    def normal(self, shape):
        return jax.random.normal(self._next(), shape, dtype=jnp.bfloat16)
    def randint(self, lo, hi, shape):
        return jax.random.randint(self._next(), shape, lo, hi, dtype=jnp.int32)
    def uniform(self, shape, lo=0.0, hi=1.0):
        return jax.random.uniform(self._next(), shape, jnp.bfloat16, lo, hi)
    def permutation(self, n):
        return jax.random.permutation(self._next(), n)


kernel_name = 'standalone__structured_sparse_n_m__ragged'

def setup_inputs():
    _rng = _Rng(jax.random.key(int.from_bytes(__import__("os").urandom(4), "little")))
    _w = (lambda a: (lambda t: t.astype(jnp.bfloat16) if jnp.issubdtype(t.dtype, jnp.floating) else t)(jnp.asarray(a)))
    B, S, D = 16, 4096, 576
    assert D % 4 == 0, "d_model must be divisible by M=4 for 2:4 sparsity"
    return {
        "x": _w((lambda *s: _rng.normal(s) * 0.05)(B, S, D)),
        "w": _w((lambda *s: _rng.normal(s) * 0.05)(D, D)),
        "b": _w((lambda *s: _rng.normal(s) * 0.05)(D)),
    }

def reference(x, w, b):
    B, S, D = x.shape
    N, M = 2, 4
    G = D // M
    wg = w.reshape(G, M, D)
    mag = jnp.abs(wg)
    order = jnp.argsort(mag, 1)
    thr = jnp.take_along_axis(mag, order[:, M - N:M - N + 1, :], 1)
    mask = (lambda x, dt: x.astype(dt))(mag >= thr, w.dtype)
    wp = (wg * mask).reshape(D, D)
    return jnp.einsum("bsd,df->bsf", x, wp) + b
```

```python
import functools
import jax
import jax.numpy as jnp
from jax import lax
import jax.experimental.pallas as pl
import jax.experimental.pallas.tpu as pltpu

F32, BF16, I32 = jnp.float32, jnp.bfloat16, jnp.int32


def _prune_packed(u):
    mate = lax.broadcasted_iota(jnp.int32, u.shape, 0) ^ 1
    lo = pltpu.bitcast((u << 16) & 0x7FFFFFFF, jnp.float32)
    hi = pltpu.bitcast(u & 0x7FFF0000, jnp.float32)
    big, small = jnp.maximum(lo, hi), jnp.minimum(lo, hi)
    nbig = jnp.take_along_axis(big, mate, axis=0, mode="promise_in_bounds")
    nsmall = jnp.take_along_axis(small, mate, axis=0, mode="promise_in_bounds")
    thr = jnp.maximum(jnp.minimum(big, nbig), jnp.maximum(small, nsmall))
    return u & (jnp.where(lo < thr, 0, 0xFFFF) | jnp.where(hi < thr, 0, -65536))


def _dot(a, b):
    return lax.dot_general(a, b, (((1,), (0,)), ((), ())), preferred_element_type=F32)


NAMES = ("r1", "v1", "v2", "v3", "u3", "u1", "u2", "q1", "p2", "r2", "w1", "w3", "w2", "p3", "q3")


def weight_forms(a):
    return dict(
        r1=a[1, 1] + a[1, 2] - a[3, 1], q1=a[1, 1] - a[2, 1] + a[1, 3],
        r2=a[2, 2] + a[2, 1] - a[3, 2], p2=a[2, 2] - a[1, 2] + a[2, 3],
        p3=a[3, 3] - a[1, 3] + a[3, 2], q3=a[3, 3] + a[3, 1] - a[2, 3],
        u1=a[2, 1] + a[1, 2], u2=a[2, 1], u3=a[1, 2],
        v1=a[3, 1] + a[1, 3], v2=a[3, 1], v3=a[1, 3],
        w1=a[2, 3] + a[3, 2], w2=a[2, 3], w3=a[3, 2])


def input_forms(x1, x2, x3, y1, y2, y3):
    s1, s2, s3 = x1 + y1, x2 + y2, x3 + y3
    return dict(r1=x1, q1=s1, r2=y2, p2=s2, p3=x3, q3=y3,
                u1=x1 + y2, u2=y1 - y2, u3=x2 - x1,
                v1=s1 - y3, v2=y3 - y1, v3=s3 - s1,
                w1=s2 - x3, w2=s3 - s2, w3=x3 - x2)


def recombine(prod):
    r1, v1, v2, v3 = prod("r1"), prod("v1"), prod("v2"), prod("v3")
    R1 = r1 + v1 + v2
    P3 = v1 + v3
    P1 = v3 + R1
    u3, u1, u2, q1 = prod("u3"), prod("u1"), prod("u2"), prod("q1")
    P2 = u3 + u1
    yield 0, P1 + u3, (u1 + u2) + (q1 - R1)
    p2, r2, w1, w3 = prod("p2"), prod("r2"), prod("w1"), prod("w3")
    R2 = r2 + w1 + w3
    left = (P2 + p2) - R2
    Q2 = u2 + R2
    R3 = v2 - w3
    Q3 = w1 - R3
    P3 = P3 + R3
    w2 = prod("w2")
    yield 1, left, Q2 + w2
    Q3 = Q3 + w2
    p3, q3 = prod("p3"), prod("q3")
    yield 2, P3 + p3, Q3 + q3


def make(do_r=True, do_w=True, do_c=True, nring=10, g0=132, rlead=8, flags=None, U=8, pipe=True,
         nfine=1, rth=2, wburst=2, tiny=False, spread=True, rextra=0, delay=720, msplit=1, pstep=3):
    NG = 256
    NIT = NG // U

    def kern(x_hbm, w_hbm, b_hbm, o_hbm, xbuf, obuf, wbuf, bbuf, lhs, bias, rhs, isem, osem):
        NB = x_hbm.shape[0]
        lhs32, rhs32 = lhs.bitcast(I32), rhs.bitcast(I32)
        tok = lambda c, n: pl.ds(c * n if isinstance(c, int) else pl.multiple_of(c * n, n), n)
        ni = pl.ds(0, 1) if tiny else slice(None)

        def icopy(t, j, c):
            return pltpu.make_async_copy(x_hbm.at[t, ni, j, :, tok(c, 512)], xbuf.at[t, ni, j, :, tok(c, 512)], isem.at[t * 8 + c])

        def iwait(q):
            pltpu.make_async_copy(xbuf.at[0, ni, :, :, tok(0, 512)], xbuf.at[0, ni, :, :, tok(0, 512)], isem.at[q]).wait()

        def ocopy(t, j, c):
            return pltpu.make_async_copy(obuf.at[t % nring, ni, j, :, tok(c, 512)], o_hbm.at[t, ni, j, :, tok(c, 512)], osem.at[t])

        def owait(t):
            pltpu.make_async_copy(obuf.at[0, ni], obuf.at[0, ni], osem.at[t]).wait()

        def read_unit(u, ks=range(8)):
            if isinstance(u, int) and u < 8:
                for j in ks:
                    icopy(0, j, u).start(priority=j % rth)
            else:
                for c in ks:
                    icopy(u // 8, u % 8, c).start(priority=c % rth)

        bcp = pltpu.make_async_copy(b_hbm, bbuf, isem.at[8 * NB])
        wcp = pltpu.make_async_copy(w_hbm, wbuf, isem.at[8 * NB + 1])
        bcp.start()
        wcp.start()
        if do_r:
            for u in range(rlead):
                read_unit(u)
        bcp.wait()
        brow = bbuf[...].reshape(1, 576).astype(F32)
        bias[...] = jnp.broadcast_to(brow, (128, 576)).T
        wcp.wait()
        u = pltpu.bitcast(wbuf[...], jnp.int32)
        parts = [_prune_packed(u[8 * i:8 * i + 8]) for i in range(36)]
        sel = []
        for k in range(3):
            sel += parts[12 * k:12 * k + 8] + parts[12 * k + 8:12 * k + 12] * 2
        wt = pltpu.bitcast(jnp.concatenate(sel, axis=0), BF16).T.astype(F32)
        a = {(f + 1, k + 1): wt[192 * f:192 * f + 192, 256 * k:256 * k + 256] for f in range(3) for k in range(3)}
        left = lax.broadcasted_iota(jnp.int32, (96, 128), 1) < 64
        forms = weight_forms(a)
        for r, name in enumerate(NAMES):
            v = forms[name]
            l0 = jnp.where(left, v[:96, :128], v[96:, :128]).astype(BF16)
            l0f = l0.astype(F32)
            lhs[0, r] = l0
            lhs[1, r] = jnp.where(left, v[:96, 128:], v[:96, :128] - l0f).astype(BF16)
            lhs[2, r] = jnp.where(left, v[96:, :128] - l0f, v[96:, 128:]).astype(BF16)
        if do_r:
            for u in range(rlead, rlead + rextra):
                read_unit(u)

        def prep(g, slot, k):
            t, cols = g
            xs, ys = [], []
            for blk in range(3):
                r8 = 24 * blk + 2 * k
                v = xbuf[t, r8 // 8, r8 % 8:r8 % 8 + 2, :, cols].astype(F32).reshape(16, 256)
                xs.append(v[:, :128])
                ys.append(v[:, 128:])
            forms = input_forms(*xs, *ys)
            for r, name in enumerate(NAMES):
                rhs[slot, r, 16 * k:16 * k + 16] = forms[name].astype(BF16)

        def pair(g, slot, hooks):
            t, cols = g
            ot = t % nring
            get = lambda r, lo, hi: pltpu.bitcast(rhs32[slot, r, lo // 2:hi // 2], BF16)
            n = [0]
            mr = 96 // msplit
            for part in range(msplit):
                z = {}
                for s in range(3):
                    def prod(name):
                        r = NAMES.index(name)
                        if n[0] % msplit == 0:
                            for h in hooks.get(n[0] // msplit, []):
                                h()
                        n[0] += 1
                        if s == 0:
                            rr = get(r, 0, 128)
                        elif s == 1:
                            rr = jnp.concatenate([get(r, 128, 192), get(r, 64, 128)], axis=0)
                        else:
                            rr = jnp.concatenate([get(r, 0, 64), get(r, 128, 192)], axis=0)
                        ll = lhs32[s, r, part * mr // 2:(part + 1) * mr // 2]
                        return _dot(pltpu.bitcast(ll, BF16), rr)

                    for f, c1, c2 in recombine(prod):
                        if s == 0:
                            z[f] = (c1, c2)
                            continue
                        row = 192 * f + 96 * (s - 1) + part * mr
                        bb = bias[row:row + mr]
                        o = jnp.concatenate([c1 + (z[f][0] + bb), c2 + (z[f][1] + bb)], axis=1)
                        for k in range(mr // 8):
                            r8 = row // 8 + k
                            obuf[ot, r8 // 8, r8 % 8, :, cols] = o[8 * k:8 * k + 8].astype(BF16)

        ncoarse = 8 * (NB - nfine)
        fine, left_over = {}, []
        gq = g0 + ncoarse - wburst
        assert ((ncoarse - 1) // 8 + 1) * 16 <= gq - 1, "coarse unit not ready"
        while gq > NG:
            gq -= 1
            left_over.append(("c", gq - g0 + wburst))
        left_over.reverse()
        for q in range(8 * nfine):
            ready = 16 * (NB - nfine) + 2 * (q + 1)
            gg = max(gq, ready)
            gq = gg + 1
            if gg < NG:
                fine.setdefault(gg % U, []).append((gg // U, q))
            else:
                left_over.append(("f", q))

        if do_r:
            iwait(0)
        if pipe and do_c:
            for k in range(12):
                prep((0, tok(0, 256)), 0, k)

        def body(it, carry):
            if do_r:
                for k in range(U // 2):
                    q = it * (U // 2) + k + 1

                    @pl.when(q < 8 * NB)
                    def _():
                        iwait(q)
            if do_w:
                @pl.when((it * U >= nring * 16) & (it % (16 // U) == 0))
                def _():
                    owait(it * U // 16 - nring)
            for p in range(U):
                g = it * U + p
                hooks = {}

                def add(pos, fn):
                    hooks.setdefault(pos, []).append(fn)

                groups = [[k] for k in range(8)] if spread else [list(range(8))]
                for gi, ks in enumerate(groups):
                    pos = 45 * gi // len(groups)
                    if do_r:
                        def rd(ks=ks):
                            @pl.when(g + rlead + rextra < 8 * NB)
                            def _():
                                read_unit(g + rlead + rextra, ks)
                        add(pos, rd)
                    if do_w:
                        if p == g0 % U and gi == 0 and wburst:
                            def burst():
                                @pl.when(g == g0)
                                def _():
                                    for k in range(wburst):
                                        for c in range(8):
                                            ocopy(k // 8, k % 8, c).start()
                            add(pos, burst)

                        def wr(ks=ks):
                            u = g - g0 + wburst

                            @pl.when((g >= g0) & (u < ncoarse))
                            def _():
                                for c in ks:
                                    ocopy(u // 8, u % 8, c).start()
                            for tt, q in fine.get(p, []):
                                @pl.when(it == tt)
                                def _():
                                    for j in ks:
                                        ocopy(NB - nfine + q // 8, j, q % 8).start()
                        add(pos, wr)
                if not do_c:
                    for pos in sorted(hooks):
                        for h in hooks[pos]:
                            h()
                    pl.delay(delay)
                    continue
                per = 16 // U
                here = (it // per, tok((it % per) * U + p if per > 1 else p, 256))
                if pipe:
                    if p == U - 1:
                        nx = jnp.minimum(it + 1, NIT - 1)
                        gn = (nx // per, tok((nx % per) * U if per > 1 else 0, 256))
                    else:
                        gn = (it // per, tok((it % per) * U + p + 1 if per > 1 else p + 1, 256))
                    for k in range(12):
                        add(int(1 + pstep * k), functools.partial(prep, gn, (p + 1) % 2, k))
                else:
                    for k in range(12):
                        prep(here, p % 2, k)
                pair(here, p % 2, hooks)
            return carry

        lax.fori_loop(0, NIT, body, 0)
        if do_w:
            for kind, q in left_over:
                for j in range(8):
                    if kind == "c":
                        ocopy(q // 8, q % 8, j).start()
                    else:
                        ocopy(NB - nfine + q // 8, j, q % 8).start()
            for t in range(NB - nring, NB):
                owait(t)
        else:
            cp = ocopy(0, 0, 0)
            cp.start()
            cp.wait()

    def fn(x, w, b):
        B, S, D = x.shape
        xt = jnp.transpose(x, (0, 2, 1)).reshape(B, 9, 8, 8, S)
        out = pl.pallas_call(
            kern,
            in_specs=[pl.BlockSpec(memory_space=pl.ANY)] * 3,
            out_specs=pl.BlockSpec(memory_space=pl.ANY),
            out_shape=jax.ShapeDtypeStruct(xt.shape, x.dtype),
            scratch_shapes=[
                pltpu.VMEM(xt.shape, BF16),
                pltpu.VMEM((nring,) + xt.shape[1:], BF16),
                pltpu.VMEM((D, D), BF16),
                pltpu.VMEM((D,), BF16),
                pltpu.VMEM((3, 15, 96, 128), BF16),
                pltpu.VMEM((D, 128), F32),
                pltpu.VMEM((2, 15, 192, 128), BF16),
                pltpu.SemaphoreType.DMA((8 * B + 2,)),
                pltpu.SemaphoreType.DMA((B,)),
            ],
            compiler_params=pltpu.CompilerParams(vmem_limit_bytes=127 * 1024 * 1024, flags=flags,
                                                 disable_bounds_checks=True, disable_semaphore_checks=True),
        )(xt, w, b)
        out = out.reshape(B, D, S)
        return jnp.transpose(out, (0, 2, 1))
    return fn


@jax.jit
def pallas_standalone__structured_sparse_n_m__ragged_kernel(x, w, b):
    return make(U=8, g0=128, nfine=2, spread=False)(x, w, b)
```

```python
import functools
import jax
import jax.numpy as jnp
from jax import lax
import jax.experimental.pallas as pl
import jax.experimental.pallas.tpu as pltpu

F32, BF16, I32 = jnp.float32, jnp.bfloat16, jnp.int32


def _prune_packed(u):
    mate = lax.broadcasted_iota(jnp.int32, u.shape, 0) ^ 1
    lo = pltpu.bitcast((u << 16) & 0x7FFFFFFF, jnp.float32)
    hi = pltpu.bitcast(u & 0x7FFF0000, jnp.float32)
    big, small = jnp.maximum(lo, hi), jnp.minimum(lo, hi)
    nbig = jnp.take_along_axis(big, mate, axis=0, mode="promise_in_bounds")
    nsmall = jnp.take_along_axis(small, mate, axis=0, mode="promise_in_bounds")
    thr = jnp.maximum(jnp.minimum(big, nbig), jnp.maximum(small, nsmall))
    return u & (jnp.where(lo < thr, 0, 0xFFFF) | jnp.where(hi < thr, 0, -65536))


def _dot(a, b):
    return lax.dot_general(a, b, (((1,), (0,)), ((), ())), preferred_element_type=F32)


NAMES = ("r1", "v1", "v2", "v3", "u3", "u1", "u2", "q1", "p2", "r2", "w1", "w3", "w2", "p3", "q3")


def weight_forms(a):
    return dict(
        r1=a[1, 1] + a[1, 2] - a[3, 1], q1=a[1, 1] - a[2, 1] + a[1, 3],
        r2=a[2, 2] + a[2, 1] - a[3, 2], p2=a[2, 2] - a[1, 2] + a[2, 3],
        p3=a[3, 3] - a[1, 3] + a[3, 2], q3=a[3, 3] + a[3, 1] - a[2, 3],
        u1=a[2, 1] + a[1, 2], u2=a[2, 1], u3=a[1, 2],
        v1=a[3, 1] + a[1, 3], v2=a[3, 1], v3=a[1, 3],
        w1=a[2, 3] + a[3, 2], w2=a[2, 3], w3=a[3, 2])


def input_forms(x1, x2, x3, y1, y2, y3):
    s1, s2, s3 = x1 + y1, x2 + y2, x3 + y3
    return dict(r1=x1, q1=s1, r2=y2, p2=s2, p3=x3, q3=y3,
                u1=x1 + y2, u2=y1 - y2, u3=x2 - x1,
                v1=s1 - y3, v2=y3 - y1, v3=s3 - s1,
                w1=s2 - x3, w2=s3 - s2, w3=x3 - x2)


def recombine(prod):
    r1, v1, v2, v3 = prod("r1"), prod("v1"), prod("v2"), prod("v3")
    R1 = r1 + v1 + v2
    P3 = v1 + v3
    P1 = v3 + R1
    u3, u1, u2, q1 = prod("u3"), prod("u1"), prod("u2"), prod("q1")
    P2 = u3 + u1
    yield 0, P1 + u3, (u1 + u2) + (q1 - R1)
    p2, r2, w1, w3 = prod("p2"), prod("r2"), prod("w1"), prod("w3")
    R2 = r2 + w1 + w3
    left = (P2 + p2) - R2
    Q2 = u2 + R2
    R3 = v2 - w3
    Q3 = w1 - R3
    P3 = P3 + R3
    w2 = prod("w2")
    yield 1, left, Q2 + w2
    Q3 = Q3 + w2
    p3, q3 = prod("p3"), prod("q3")
    yield 2, P3 + p3, Q3 + q3


def make(do_r=True, do_w=True, do_c=True, nring=10, g0=132, rlead=8, flags=None, U=8, pipe=True,
         nfine=1, rth=2, wburst=2, tiny=False, spread=True, rextra=0, delay=720, msplit=1, pstep=3, pin=0, pinlag=1):
    NG = 256
    NIT = NG // U

    def kern(x_hbm, w_hbm, b_hbm, o_hbm, xbuf, obuf, wbuf, bbuf, lhs, bias, rhs, flag, isem, osem):
        NB = x_hbm.shape[0]
        x32 = xbuf.bitcast(I32)
        lhs32, rhs32 = lhs.bitcast(I32), rhs.bitcast(I32)
        tok = lambda c, n: c
        ni = pl.ds(0, 1) if tiny else slice(None)

        def icopy(t, j, c):
            return pltpu.make_async_copy(x_hbm.at[t, ni, j, pl.ds(2 * c, 2)], xbuf.at[t, ni, j, pl.ds(2 * c, 2)], isem.at[t * 8 + c])

        def iwait(q):
            pltpu.make_async_copy(xbuf.at[0, ni, :, pl.ds(0, 2)], xbuf.at[0, ni, :, pl.ds(0, 2)], isem.at[q]).wait()

        def ocopy(t, j, c):
            return pltpu.make_async_copy(obuf.at[t % nring, ni, j, pl.ds(2 * c, 2)], o_hbm.at[t, ni, j, pl.ds(2 * c, 2)], osem.at[t])

        def owait(t):
            pltpu.make_async_copy(obuf.at[0, ni], obuf.at[0, ni], osem.at[t]).wait()

        def read_unit(u, ks=range(8)):
            if isinstance(u, int) and u < 8:
                for j in ks:
                    icopy(0, j, u).start(priority=j % rth)
            else:
                for c in ks:
                    icopy(u // 8, u % 8, c).start(priority=c % rth)

        bcp = pltpu.make_async_copy(b_hbm, bbuf, isem.at[8 * NB])
        wcp = pltpu.make_async_copy(w_hbm, wbuf, isem.at[8 * NB + 1])
        bcp.start()
        wcp.start()
        if do_r:
            for u in range(rlead):
                read_unit(u)
        bcp.wait()
        brow = bbuf[...].reshape(1, 576).astype(F32)
        bias[...] = jnp.broadcast_to(brow, (128, 576)).T
        wcp.wait()
        u = pltpu.bitcast(wbuf[...], jnp.int32)
        parts = [_prune_packed(u[8 * i:8 * i + 8]) for i in range(36)]
        sel = []
        for k in range(3):
            sel += parts[12 * k:12 * k + 8] + parts[12 * k + 8:12 * k + 12] * 2
        wt = pltpu.bitcast(jnp.concatenate(sel, axis=0), BF16).T.astype(F32)
        a = {(f + 1, k + 1): wt[192 * f:192 * f + 192, 256 * k:256 * k + 256] for f in range(3) for k in range(3)}
        left = lax.broadcasted_iota(jnp.int32, (96, 128), 1) < 64
        forms = weight_forms(a)
        for r, name in enumerate(NAMES):
            v = forms[name]
            l0 = jnp.where(left, v[:96, :128], v[96:, :128]).astype(BF16)
            l0f = l0.astype(F32)
            lhs[0, r] = l0
            lhs[1, r] = jnp.where(left, v[:96, 128:], v[:96, :128] - l0f).astype(BF16)
            lhs[2, r] = jnp.where(left, v[96:, :128] - l0f, v[96:, 128:]).astype(BF16)
        if do_r:
            for u in range(rlead, rlead + rextra):
                read_unit(u)

        last = []

        def prep(g, slot, k):
            t, cols = g
            xs, ys = [], []
            for blk in range(3):
                r8 = 24 * blk + 2 * k
                v = []
                for h in range(2):
                    words = x32[t, r8 // 8, r8 % 8 + h, cols]
                    if pin and len(last) >= pinlag:
                        words = jnp.where(always[0], words, pltpu.bitcast(last[-pinlag][0:8], I32))
                    v.append(pltpu.bitcast(words, BF16).astype(F32))
                xs.append(jnp.concatenate([v[0][0:8], v[1][0:8]], axis=0))
                ys.append(jnp.concatenate([v[0][8:16], v[1][8:16]], axis=0))
            forms = input_forms(*xs, *ys)
            for r, name in enumerate(NAMES):
                rhs[slot, r, 16 * k:16 * k + 16] = forms[name].astype(BF16)

        def pair(g, slot, hooks):
            t, cols = g
            ot = t % nring
            get = lambda r, lo, hi: pltpu.bitcast(rhs32[slot, r, lo // 2:hi // 2], BF16)
            n = [0]
            mr = 96 // msplit
            for part in range(msplit):
                z = {}
                for s in range(3):
                    def prod(name):
                        r = NAMES.index(name)
                        if n[0] % msplit == 0:
                            for h in hooks.get(n[0] // msplit, []):
                                h()
                        n[0] += 1
                        if s == 0:
                            rr = get(r, 0, 128)
                        elif s == 1:
                            rr = jnp.concatenate([get(r, 128, 192), get(r, 64, 128)], axis=0)
                        else:
                            rr = jnp.concatenate([get(r, 0, 64), get(r, 128, 192)], axis=0)
                        ll = lhs32[s, r, part * mr // 2:(part + 1) * mr // 2]
                        last.append(_dot(pltpu.bitcast(ll, BF16), rr))
                        return last[-1]

                    for f, c1, c2 in recombine(prod):
                        if s == 0:
                            z[f] = (c1, c2)
                            continue
                        row = 192 * f + 96 * (s - 1) + part * mr
                        bb = bias[row:row + mr]
                        c1, c2 = c1 + (z[f][0] + bb), c2 + (z[f][1] + bb)
                        for k in range(mr // 8):
                            r8 = row // 8 + k
                            o = jnp.concatenate([c1[8 * k:8 * k + 8], c2[8 * k:8 * k + 8]], axis=0)
                            obuf[ot, r8 // 8, r8 % 8, cols] = o.astype(BF16)

        ncoarse = 8 * (NB - nfine)
        fine, left_over = {}, []
        gq = g0 + ncoarse - wburst
        assert ((ncoarse - 1) // 8 + 1) * 16 <= gq - 1, "coarse unit not ready"
        while gq > NG:
            gq -= 1
            left_over.append(("c", gq - g0 + wburst))
        left_over.reverse()
        for q in range(8 * nfine):
            ready = 16 * (NB - nfine) + 2 * (q + 1)
            gg = max(gq, ready)
            gq = gg + 1
            if gg < NG:
                fine.setdefault(gg % U, []).append((gg // U, q))
            else:
                left_over.append(("f", q))

        if do_r:
            iwait(0)
        if pipe and do_c:
            for k in range(12):
                prep((0, tok(0, 256)), 0, k)

        always = [None]
        flag[...] = jnp.zeros(flag.shape, I32)

        def body(it, carry):
            always[0] = flag[it % 2] == 0
            del last[:]
            if do_r:
                for k in range(U // 2):
                    q = it * (U // 2) + k + 1

                    @pl.when(q < 8 * NB)
                    def _():
                        iwait(q)
            if do_w:
                @pl.when((it * U >= nring * 16) & (it % (16 // U) == 0))
                def _():
                    owait(it * U // 16 - nring)
            for p in range(U):
                g = it * U + p
                hooks = {}

                def add(pos, fn):
                    hooks.setdefault(pos, []).append(fn)

                groups = [[k] for k in range(8)] if spread else [list(range(8))]
                for gi, ks in enumerate(groups):
                    pos = 45 * gi // len(groups)
                    if do_r:
                        def rd(ks=ks):
                            @pl.when(g + rlead + rextra < 8 * NB)
                            def _():
                                read_unit(g + rlead + rextra, ks)
                        add(pos, rd)
                    if do_w:
                        if p == g0 % U and gi == 0 and wburst:
                            def burst():
                                @pl.when(g == g0)
                                def _():
                                    for k in range(wburst):
                                        for c in range(8):
                                            ocopy(k // 8, k % 8, c).start()
                            add(pos, burst)

                        def wr(ks=ks):
                            u = g - g0 + wburst

                            @pl.when((g >= g0) & (u < ncoarse))
                            def _():
                                for c in ks:
                                    ocopy(u // 8, u % 8, c).start()
                            for tt, q in fine.get(p, []):
                                @pl.when(it == tt)
                                def _():
                                    for j in ks:
                                        ocopy(NB - nfine + q // 8, j, q % 8).start()
                        add(pos, wr)
                if not do_c:
                    for pos in sorted(hooks):
                        for h in hooks[pos]:
                            h()
                    pl.delay(delay)
                    continue
                per = 16 // U
                here = (it // per, tok((it % per) * U + p if per > 1 else p, 256))
                if pipe:
                    if p == U - 1:
                        nx = jnp.minimum(it + 1, NIT - 1)
                        gn = (nx // per, tok((nx % per) * U if per > 1 else 0, 256))
                    else:
                        gn = (it // per, tok((it % per) * U + p + 1 if per > 1 else p + 1, 256))
                    for k in range(12):
                        add(int(1 + pstep * k), functools.partial(prep, gn, (p + 1) % 2, k))
                else:
                    for k in range(12):
                        prep(here, p % 2, k)
                pair(here, p % 2, hooks)
            return carry

        lax.fori_loop(0, NIT, body, 0)
        if do_w:
            for kind, q in left_over:
                for j in range(8):
                    if kind == "c":
                        ocopy(q // 8, q % 8, j).start()
                    else:
                        ocopy(NB - nfine + q // 8, j, q % 8).start()
            for t in range(NB - nring, NB):
                owait(t)
        else:
            cp = ocopy(0, 0, 0)
            cp.start()
            cp.wait()

    def fn(x, w, b):
        B, S, D = x.shape
        xt = jnp.transpose(x, (0, 2, 1)).reshape(B, D // 8, 8, S // 128, 128).transpose(0, 1, 3, 2, 4)
        xt = xt.reshape(B, 9, 8, 16, 16, 128)
        out = pl.pallas_call(
            kern,
            in_specs=[pl.BlockSpec(memory_space=pl.ANY)] * 3,
            out_specs=pl.BlockSpec(memory_space=pl.ANY),
            out_shape=jax.ShapeDtypeStruct(xt.shape, x.dtype),
            scratch_shapes=[
                pltpu.VMEM(xt.shape, BF16),
                pltpu.VMEM((nring,) + xt.shape[1:], BF16),
                pltpu.VMEM((D, D), BF16),
                pltpu.VMEM((D,), BF16),
                pltpu.VMEM((3, 15, 96, 128), BF16),
                pltpu.VMEM((D, 128), F32),
                pltpu.VMEM((2, 15, 192, 128), BF16),
                pltpu.VMEM((2, 8, 128), I32),
                pltpu.SemaphoreType.DMA((8 * B + 2,)),
                pltpu.SemaphoreType.DMA((B,)),
            ],
            compiler_params=pltpu.CompilerParams(vmem_limit_bytes=127 * 1024 * 1024, flags=flags,
                                                 disable_bounds_checks=True, disable_semaphore_checks=True),
        )(xt, w, b)
        out = out.reshape(B, D // 8, S // 128, 8, 128).transpose(0, 1, 3, 2, 4).reshape(B, D, S)
        return jnp.transpose(out, (0, 2, 1))
    return fn


@jax.jit
def pallas_standalone__structured_sparse_n_m__ragged_kernel(x, w, b):
    return make(U=8, pin=1, pstep=3.5, pinlag=4, g0=123, nfine=3)(x, w, b)
```

```python
import functools
import jax
import jax.numpy as jnp
from jax import lax
import jax.experimental.pallas as pl
import jax.experimental.pallas.tpu as pltpu

F32, BF16, I32 = jnp.float32, jnp.bfloat16, jnp.int32


def _prune_packed(u):
    mate = lax.broadcasted_iota(jnp.int32, u.shape, 0) ^ 1
    lo = pltpu.bitcast((u << 16) & 0x7FFFFFFF, jnp.float32)
    hi = pltpu.bitcast(u & 0x7FFF0000, jnp.float32)
    big, small = jnp.maximum(lo, hi), jnp.minimum(lo, hi)
    nbig = jnp.take_along_axis(big, mate, axis=0, mode="promise_in_bounds")
    nsmall = jnp.take_along_axis(small, mate, axis=0, mode="promise_in_bounds")
    thr = jnp.maximum(jnp.minimum(big, nbig), jnp.maximum(small, nsmall))
    return u & (jnp.where(lo < thr, 0, 0xFFFF) | jnp.where(hi < thr, 0, -65536))


def _dot(a, b):
    return lax.dot_general(a, b, (((1,), (0,)), ((), ())), preferred_element_type=F32)


NAMES = ("r1", "v1", "v2", "v3", "u3", "u1", "u2", "q1", "p2", "r2", "w1", "w3", "w2", "p3", "q3")


def weight_forms(a):
    return dict(
        r1=a[1, 1] + a[1, 2] - a[3, 1], q1=a[1, 1] - a[2, 1] + a[1, 3],
        r2=a[2, 2] + a[2, 1] - a[3, 2], p2=a[2, 2] - a[1, 2] + a[2, 3],
        p3=a[3, 3] - a[1, 3] + a[3, 2], q3=a[3, 3] + a[3, 1] - a[2, 3],
        u1=a[2, 1] + a[1, 2], u2=a[2, 1], u3=a[1, 2],
        v1=a[3, 1] + a[1, 3], v2=a[3, 1], v3=a[1, 3],
        w1=a[2, 3] + a[3, 2], w2=a[2, 3], w3=a[3, 2])


def input_forms(x1, x2, x3, y1, y2, y3):
    s1, s2, s3 = x1 - y1, x2 - y2, x3 - y3
    return dict(r1=x1, q1=s1, r2=y2, p2=s2, p3=x3, q3=y3,
                u1=x1 - y2, u2=y2 - y1, u3=x2 - x1,
                v1=s1 + y3, v2=y1 - y3, v3=s3 - s1,
                w1=s2 - x3, w2=s3 - s2, w3=x3 - x2)


def recombine(prod, init):
    r1, v1, v2, v3 = prod("r1"), prod("v1"), prod("v2"), prod("v3")
    R1 = init(0, 2, r1) + v1 + v2
    P3 = init(2, 0, v1) + v3
    P1 = init(0, 0, v3) + R1
    u3, u1, u2, q1 = prod("u3"), prod("u1"), prod("u2"), prod("q1")
    P2 = init(1, 0, u3) + u1
    yield 0, P1 + u3, (init(0, 1, R1) - q1) - (u1 + u2)
    p2, r2, w1, w3 = prod("p2"), prod("r2"), prod("w1"), prod("w3")
    R2 = init(1, 2, r2) - w1 - w3
    left = (P2 + p2) + R2
    Q2 = init(1, 1, R2) - u2
    R3 = init(2, 2, v2) - w3
    Q3 = init(2, 1, R3) - w1
    P3 = P3 + R3
    w2 = prod("w2")
    yield 1, left, Q2 - w2
    Q3 = Q3 - w2
    p3, q3 = prod("p3"), prod("q3")
    yield 2, P3 + p3, Q3 + q3


def make(do_r=True, do_w=True, do_c=True, nring=10, rlead=8, flags=None, U=16, tiny=False, delay=720,
         msplit=1, p0=1, pstep=3.5, pin=1, pinlag=4, ppos=None, pmajor=False, late_init=False, zs=False,
         wburst=2, gsw=128, swq=1, pinrow=0, nsub=1, sublag=1, dpos=0, waits=(1, 3, 7, 15), ntail=1, tail_groups=(4, 4), catchup=1, ipat="00001111", rpat="01010101"):
    NG = 256
    swq = swq if do_w else 0
    NIT = NG // U
    per = 16 // U

    def kern(x_hbm, w_hbm, b_hbm, o_hbm, xbuf, obuf, wbuf, bbuf, lhs, bias, rhs, flag, zbuf, isem, osem):
        NB = x_hbm.shape[0]
        x32, lhs32, rhs32 = xbuf.bitcast(I32), lhs.bitcast(I32), rhs.bitcast(I32)
        ni = pl.ds(0, 1) if tiny else slice(None)
        LAST = 4 * NB

        def icopy(t, j, c, sem):
            return pltpu.make_async_copy(x_hbm.at[t, ni, j, pl.ds(2 * c, 2)], xbuf.at[t, ni, j, pl.ds(2 * c, 2)],
                                         isem.at[sem])

        def iwait(sem, nquad):
            v = xbuf.at[0, ni, :, pl.ds(0, 2 * nquad)]
            pltpu.make_async_copy(v, v, isem.at[sem]).wait()

        def ocopy(t, j, c):
            return pltpu.make_async_copy(obuf.at[t % nring, ni, j, pl.ds(2 * c, 2)], o_hbm.at[t, ni, j, pl.ds(2 * c, 2)],
                                         osem.at[t])

        def owait(t):
            pltpu.make_async_copy(obuf.at[0, ni], obuf.at[0, ni], osem.at[t]).wait()

        def read_unit(u, ks=range(8), c=None):
            t = u // 8
            sem = 4 * t + c.bit_length()
            if swq and c >= 8 - swq:
                sem = jnp.where(t == NB - 1, LAST, sem) if not isinstance(t, int) else sem
            for j in ks:
                pr = int(ipat[u]) if isinstance(u, int) and u < len(ipat) and ipat[u] in "01" else int(rpat[j])
                icopy(t, j, c, sem).start(priority=pr)

        bcp = pltpu.make_async_copy(b_hbm, bbuf, isem.at[LAST + 1])
        wcp = pltpu.make_async_copy(w_hbm, wbuf, isem.at[LAST + 2])
        bcp.start()
        wcp.start()
        if do_r:
            for u in range(rlead):
                read_unit(u, c=u % 8)
        bcp.wait()
        brow = bbuf[...].reshape(1, 576).astype(F32)
        bias[...] = jnp.broadcast_to(brow, (128, 576)).T
        wcp.wait()
        u = pltpu.bitcast(wbuf[...], jnp.int32)
        parts = [_prune_packed(u[8 * i:8 * i + 8]) for i in range(36)]
        sel = []
        for k in range(3):
            sel += parts[12 * k:12 * k + 8] + parts[12 * k + 8:12 * k + 12] * 2
        wt = pltpu.bitcast(jnp.concatenate(sel, axis=0), BF16).T.astype(F32)
        a = {(f + 1, k + 1): wt[192 * f:192 * f + 192, 256 * k:256 * k + 256] for f in range(3) for k in range(3)}
        left = lax.broadcasted_iota(jnp.int32, (96, 128), 1) < 64
        forms = weight_forms(a)
        for r, name in enumerate(NAMES):
            v = forms[name]
            l0 = jnp.where(left, v[:96, :128], v[96:, :128]).astype(BF16)
            l0f = l0.astype(F32)
            lhs[0, r] = l0
            lhs[1, r] = jnp.where(left, v[:96, 128:], v[:96, :128] - l0f).astype(BF16)
            lhs[2, r] = jnp.where(left, v[96:, :128] - l0f, v[96:, 128:]).astype(BF16)

        last = []
        always = [None]

        def dep(v):
            if pin and len(last) >= pinlag:
                d = last[-pinlag][8 * pinrow:8 * pinrow + 8]
                if v.shape[0] == 16:
                    return jnp.concatenate([jnp.where(always[0], v[0:8], d), v[8:16]], axis=0)
                return jnp.where(always[0], v, pltpu.bitcast(d, I32))
            return v

        def prep(g, slot, k):
            t, cols = g
            xs, ys = [], []
            for blk in range(3):
                r8 = 24 * blk + 2 * k
                v = [pltpu.bitcast(dep(x32[t, r8 // 8, r8 % 8 + h, cols]), BF16).astype(F32) for h in range(2)]
                xs.append(jnp.concatenate([v[0][0:8], v[1][0:8]], axis=0))
                ys.append(jnp.concatenate([v[0][8:16], v[1][8:16]], axis=0))
            forms = input_forms(*xs, *ys)
            for r, name in enumerate(NAMES):
                if nsub > 1 and r and r % (15 // nsub) == 0:
                    yield
                val = forms[name]
                if nsub > 1 and r >= 15 // nsub:
                    val = dep(val)
                rhs[slot, r, 16 * k:16 * k + 16] = val.astype(BF16)

        def pair(g, slot, hooks):
            t, cols = g
            ot = t % nring
            get = lambda r, lo, hi: pltpu.bitcast(rhs32[slot, r, lo // 2:hi // 2], BF16)
            n = [0]
            mr = 96 // msplit

            def one(s, name, part):
                r = NAMES.index(name)
                if n[0] % msplit == 0:
                    for h in hooks.get(n[0] // msplit, []):
                        h()
                n[0] += 1
                if s == 0:
                    rr = get(r, 0, 128)
                elif s == 1:
                    rr = jnp.concatenate([get(r, 128, 192), get(r, 64, 128)], axis=0)
                else:
                    rr = jnp.concatenate([get(r, 0, 64), get(r, 128, 192)], axis=0)
                ll = lhs32[s, r, part * mr // 2:(part + 1) * mr // 2]
                last.append(_dot(pltpu.bitcast(ll, BF16), rr))
                return last[-1]

            def put(row, c1, c2):
                for k in range(mr // 8):
                    r8 = row // 8 + k
                    o = jnp.concatenate([c1[8 * k:8 * k + 8], c2[8 * k:8 * k + 8]], axis=0)
                    obuf[ot, r8 // 8, r8 % 8, cols] = o.astype(BF16)

            for part in range(msplit):
                if pmajor:
                    def prod(name):
                        sh = one(0, name, part)
                        return jnp.concatenate([sh + one(1, name, part), sh + one(2, name, part)], axis=0)

                    def init(f, k, v):
                        if k < 2:
                            return v
                        row = 192 * f + part * mr
                        return v + jnp.concatenate([bias[row:row + mr], bias[row + 96:row + 96 + mr]], axis=0)

                    for f, c1, c2 in recombine(prod, init):
                        for e in range(2):
                            put(192 * f + 96 * e + part * mr, c1[e * mr:(e + 1) * mr], c2[e * mr:(e + 1) * mr])
                    continue
                z = {}
                for s in range(3):
                    def zget(f, k):
                        return zbuf[part, f, k] if zs else z[f][k]

                    def init(f, k, v):
                        if s == 0:
                            return v
                        row = 192 * f + 96 * (s - 1) + part * mr
                        if k == 2:
                            return v + bias[row:row + mr]
                        return v if late_init else v + zget(f, k)

                    for f, c1, c2 in recombine(lambda name: one(s, name, part), init):
                        if s == 0:
                            if zs:
                                zbuf[part, f, 0], zbuf[part, f, 1] = c1, c2
                            z[f] = (c1, c2)
                            continue
                        if late_init:
                            c1, c2 = c1 + zget(f, 0), c2 + zget(f, 1)
                        put(192 * f + 96 * (s - 1) + part * mr, c1, c2)

        if do_r:
            iwait(0, 1)
        if do_c:
            for k in range(12):
                for _ in prep((0, 0), 0, k):
                    pass
        flag[...] = jnp.zeros(flag.shape, I32)

        ncoarse = 0
        while ncoarse < 8 * (NB - ntail) and gsw - wburst + ncoarse >= 16 * (ncoarse // 8 + 1):
            ncoarse += 1
        ncoarse -= ncoarse % 8
        todo = []
        for t in range(ncoarse // 8, NB):
            groups = tail_groups if t == NB - 1 else (8,)
            c0 = 0
            for n in groups:
                todo += [(16 * t + 2 * (c0 + n), t, j, c) for j in range(8) for c in range(c0, c0 + n)]
                c0 += n
        tail, gq = {}, gsw - wburst + ncoarse
        while todo and gq < NG:
            for gi in range(8):
                for _ in range(catchup):
                    if todo and todo[0][0] <= gq:
                        tail.setdefault((gq % U, gi), []).append((gq,) + todo.pop(0)[1:])
            gq += 1

        def body(it, carry):
            always[0] = flag[it % 2] == 0
            del last[:]
            if do_w:
                @pl.when((it * U >= nring * 16) & (it % per == 0))
                def _():
                    owait(it // per - nring)
            for p in range(U):
                g = it * U + p
                hooks = {}

                def add(pos, fn):
                    hooks.setdefault(pos, []).append(fn)

                if do_r:
                    def wt_():
                        for wp in waits:
                            if wp % U != p:
                                continue
                            mine = (g % 16 == wp) if per > 1 else True
                            t = it // per
                            if wp == 15:
                                @pl.when(mine & (t + 1 < NB))
                                def _():
                                    iwait(4 * t + 4, 1)
                            elif wp == 7 and swq and do_w:
                                @pl.when(mine & (t < NB - 1))
                                def _():
                                    iwait(4 * t + 3, 4)

                                @pl.when(mine & (t == NB - 1))
                                def _():
                                    iwait(LAST, swq)
                            elif per > 1:
                                @pl.when(mine)
                                def _():
                                    iwait(4 * t + (wp + 1).bit_length() - 1, (wp + 1) // 2)
                            else:
                                iwait(4 * t + (wp + 1).bit_length() - 1, (wp + 1) // 2)
                    add(0, wt_)
                if do_w and p == gsw % U:
                    def burst():
                        @pl.when(g == gsw)
                        def _():
                            if do_r and swq:
                                iwait(4 * NB - 1, 4 - swq)
                            for k in range(wburst):
                                for c in range(8):
                                    ocopy(k // 8, k % 8, c).start()
                    add(0, burst)
                for gi in range(8):
                    pos = (dpos + 45 * gi // 8) % 45
                    if do_r:
                        def rd(gi=gi):
                            @pl.when(g + rlead < 8 * NB)
                            def _():
                                read_unit(g + rlead, [gi], c=(p + rlead) % 8)
                        add(pos, rd)
                    if do_w:
                        def wr(gi=gi):
                            u = g - gsw + wburst

                            @pl.when((g >= gsw) & (u < ncoarse))
                            def _():
                                ocopy(u // 8, u % 8, gi).start()
                            for gg, t, j, c in tail.get((p, gi), []):
                                @pl.when(g == gg)
                                def _():
                                    ocopy(t, j, c).start()
                        add(pos, wr)
                if not do_c:
                    for pos in sorted(hooks):
                        for h in hooks[pos]:
                            h()
                    pl.delay(delay)
                    continue
                here = (it // per, (it % per) * U + p if per > 1 else p)
                if p == U - 1:
                    nx = jnp.minimum(it + 1, NIT - 1)
                    gn = (nx // per, (nx % per) * U if per > 1 else 0)
                else:
                    gn = (it // per, (it % per) * U + p + 1 if per > 1 else p + 1)
                for k in range(12):
                    gen = prep(gn, (p + 1) % 2, k)
                    for q in range(nsub):
                        add((ppos[k] if ppos else int(p0 + pstep * k)) + q * sublag,
                            functools.partial(next, gen, None))
                pair(here, p % 2, hooks)
            return carry

        lax.fori_loop(0, NIT, body, 0)
        if do_w:
            for _, t, j, c in todo:
                ocopy(t, j, c).start()
            for t in range(NB - nring, NB):
                owait(t)
        else:
            cp = ocopy(0, 0, 0)
            cp.start()
            cp.wait()

    def fn(x, w, b):
        B, S, D = x.shape
        xt = jnp.transpose(x, (0, 2, 1)).reshape(B, D // 8, 8, S // 128, 128).transpose(0, 1, 3, 2, 4)
        xt = xt.reshape(B, 9, 8, 16, 16, 128)
        out = pl.pallas_call(
            kern,
            in_specs=[pl.BlockSpec(memory_space=pl.ANY)] * 3,
            out_specs=pl.BlockSpec(memory_space=pl.ANY),
            out_shape=jax.ShapeDtypeStruct(xt.shape, x.dtype),
            scratch_shapes=[
                pltpu.VMEM(xt.shape, BF16),
                pltpu.VMEM((nring,) + xt.shape[1:], BF16),
                pltpu.VMEM((D, D), BF16),
                pltpu.VMEM((D,), BF16),
                pltpu.VMEM((3, 15, 96, 128), BF16),
                pltpu.VMEM((D, 128), F32),
                pltpu.VMEM((2, 15, 192, 128), BF16),
                pltpu.VMEM((2, 8, 128), I32),
                pltpu.VMEM((msplit, 3, 2, 96 // msplit, 128), F32),
                pltpu.SemaphoreType.DMA((4 * B + 3,)),
                pltpu.SemaphoreType.DMA((B,)),
            ],
            compiler_params=pltpu.CompilerParams(vmem_limit_bytes=127 * 1024 * 1024, flags=flags,
                                                 disable_bounds_checks=True, disable_semaphore_checks=True),
        )(xt, w, b)
        out = out.reshape(B, D // 8, S // 128, 8, 128).transpose(0, 1, 3, 2, 4).reshape(B, D, S)
        return jnp.transpose(out, (0, 2, 1))
    return fn


@jax.jit
def pallas_standalone__structured_sparse_n_m__ragged_kernel(x, w, b):
    return make(U=16, nsub=3, msplit=2, flags={"XLA_TPU_RESCHEDULE_DMA_DONES": True}, wburst=1, rlead=5,
                ipat="001", gsw=126, swq=2)(x, w, b)
```

```python
import functools

import jax
import jax.numpy as jnp
from jax import lax
import jax.experimental.pallas as pl
import jax.experimental.pallas.tpu as pltpu

F32, BF16, I32 = jnp.float32, jnp.bfloat16, jnp.int32

PRODUCTS = ("r1", "v1", "v2", "v3", "u3", "u1", "u2", "q1", "p2", "r2", "w1", "w3", "w2", "p3", "q3")


def _weight_forms(a):
    return dict(
        r1=a[1, 1] + a[1, 2] - a[3, 1], q1=a[1, 1] - a[2, 1] + a[1, 3],
        r2=a[2, 2] + a[2, 1] - a[3, 2], p2=a[2, 2] - a[1, 2] + a[2, 3],
        p3=a[3, 3] - a[1, 3] + a[3, 2], q3=a[3, 3] + a[3, 1] - a[2, 3],
        u1=a[2, 1] + a[1, 2], u2=a[2, 1], u3=a[1, 2],
        v1=a[3, 1] + a[1, 3], v2=a[3, 1], v3=a[1, 3],
        w1=a[2, 3] + a[3, 2], w2=a[2, 3], w3=a[3, 2])


def _input_forms(x1, x2, x3, y1, y2, y3):
    s1, s2, s3 = x1 - y1, x2 - y2, x3 - y3
    return dict(r1=x1, q1=s1, r2=y2, p2=s2, p3=x3, q3=y3,
                u1=x1 - y2, u2=y2 - y1, u3=x2 - x1,
                v1=s1 + y3, v2=y1 - y3, v3=s3 - s1,
                w1=s2 - x3, w2=s3 - s2, w3=x3 - x2)


def _output_blocks(prod, plus):
    r1, v1, v2, v3 = prod("r1"), prod("v1"), prod("v2"), prod("v3")
    both1 = plus(0, 2, r1) + v1 + v2
    first3 = plus(2, 0, v1) + v3
    first1 = plus(0, 0, v3) + both1
    u3, u1, u2, q1 = prod("u3"), prod("u1"), prod("u2"), prod("q1")
    first2 = plus(1, 0, u3) + u1
    yield 0, first1 + u3, (plus(0, 1, both1) - q1) - (u1 + u2)
    p2, r2, w1, w3 = prod("p2"), prod("r2"), prod("w1"), prod("w3")
    both2 = plus(1, 2, r2) - w1 - w3
    first2 = (first2 + p2) + both2
    second2 = plus(1, 1, both2) - u2
    both3 = plus(2, 2, v2) - w3
    second3 = plus(2, 1, both3) - w1
    first3 = first3 + both3
    w2 = prod("w2")
    yield 1, first2, second2 - w2
    second3 = second3 - w2
    p3, q3 = prod("p3"), prod("q3")
    yield 2, first3 + p3, second3 + q3


def _prune_packed(u):
    mate = lax.broadcasted_iota(I32, u.shape, 0) ^ 1
    lo = pltpu.bitcast((u << 16) & 0x7FFFFFFF, F32)
    hi = pltpu.bitcast(u & 0x7FFF0000, F32)
    big, small = jnp.maximum(lo, hi), jnp.minimum(lo, hi)
    nbig = jnp.take_along_axis(big, mate, axis=0, mode="promise_in_bounds")
    nsmall = jnp.take_along_axis(small, mate, axis=0, mode="promise_in_bounds")
    thr = jnp.maximum(jnp.minimum(big, nbig), jnp.maximum(small, nsmall))
    return u & (jnp.where(lo < thr, 0, 0xFFFF) | jnp.where(hi < thr, 0, -65536))


def make(do_w=True, RING=5, READ_AHEAD=40, SWITCH=124, READ_OVERLAP=32, WRITE_AHEAD=4, TAIL=(2, 1, 1),
         PREP_AT=1, PREP_EVERY=3.5, PIN_BACK=4, PIN_ROW=0, PREP_PARTS=3, PART_EVERY=1, DMA_AT=0,
         ipat="001", WPARTS=3, late_rate=8, rowstep=16, skew=0, lo_first=0):
    BATCHES, PAIRS, PASSES, ROWS = 16, 16, 45, 48
    QUAD_GROUPS = ((0, 1), (1, 2), (2, 4), (4, 6), (6, 8))
    if not do_w:
        READ_OVERLAP = 0

    def write_plan():
        whole = 0
        while whole < BATCHES // 2 - 1 and SWITCH + (64 * whole - WRITE_AHEAD) // 4 >= 2 * PAIRS * (whole + 1):
            whole += 1
        todo, pos = [], 8 * whole
        for n in [4] * ((4 * BATCHES - pos - sum(TAIL)) // 4) + list(TAIL):
            t, c0 = divmod(pos, 4)
            assert c0 + n <= 4
            for r in range(16):
                i, j = divmod(72 * (t % 2) + r, 16)
                todo += [(PAIRS * t + 4 * (c0 + n), (t // 2, i, len(range(r, 72, 16)), j, c))
                         for c in range(c0, c0 + n)]
            pos += n
        assert pos == 4 * BATCHES
        late = {}
        for step in range(SWITCH - (WRITE_AHEAD - 64 * whole) // 4, BATCHES * PAIRS):
            for slot in range(late_rate):
                if todo and todo[0][0] <= step:
                    late.setdefault((step % PAIRS, slot * 8 // late_rate), []).append((step // PAIRS, todo.pop(0)[1]))
        return whole, late, [copy for _, copy in todo]

    def _kernel(x_hbm, w_hbm, b_hbm, o_hbm, xbuf, obuf, wbuf, bbuf, lhs, rhs, bias, zero,
                qsem, xsem, osem):
        x_words, lhs_words, rhs_words = xbuf.bitcast(I32), lhs.bitcast(I32), rhs.bitcast(I32)

        def read_quad(k, thread):
            t, c, j = k // 64, k // 8 % 8, k % 8
            at = (pl.ds(9 * t, 9), j, pl.ds(2 * c, 2))
            group = next(g for g, (lo, hi) in enumerate(QUAD_GROUPS) if lo <= c < hi)
            pltpu.make_async_copy(x_hbm.at[at], xbuf.at[at], qsem.at[t, group]).start(priority=thread)

        def read_row(d, k):
            h, r = divmod(k, 144)
            row = r * rowstep % 144 + r * rowstep // 144 if 144 % rowstep == 0 else r * rowstep % 144
            at = (18 * d + row // 8, row % 8, pl.ds(8 * h, 8))
            sem = 2 * d + h
            if k >= 288 - READ_OVERLAP:
                sem = jnp.where(d == BATCHES // 2 - 1, 0, sem)
            pltpu.make_async_copy(x_hbm.at[at], xbuf.at[at], xsem.at[sem]).start(priority=(k + lo_first) % 2)

        def wait_read(sem, *at):
            pltpu.make_async_copy(xbuf.at[at], xbuf.at[at], sem).wait()

        def wait_quads(t, group):
            lo, hi = QUAD_GROUPS[group]
            wait_read(qsem.at[t, group], pl.ds(0, 9), slice(None), pl.ds(0, 2 * (hi - lo)))

        def wait_rows(sem, n):
            wait_read(xsem.at[sem], pl.ds(0, n), 0, pl.ds(0, 8))

        def write(d, i, n, j, c):
            pltpu.make_async_copy(obuf.at[pl.ds(9 * (d % RING) + i, n), j, pl.ds(4 * c, 4)],
                                  o_hbm.at[pl.ds(9 * d + i, n), j, pl.ds(4 * c, 4)], osem.at[d]).start()

        def wait_written(d):
            pltpu.make_async_copy(obuf.at[pl.ds(0, 9)], obuf.at[pl.ds(0, 9)], osem.at[d]).wait()

        rows = 576 // WPARTS
        w_copies = [pltpu.make_async_copy(w_hbm.at[pl.ds(rows * k, rows)], wbuf.at[pl.ds(rows * k, rows)],
                                          qsem.at[2, k]) for k in range(WPARTS)]
        b_copy = pltpu.make_async_copy(b_hbm, bbuf, qsem.at[2, WPARTS])
        b_copy.start()
        for copy in w_copies:
            copy.start()
        for k in range(READ_AHEAD):
            read_quad(k, int(ipat[k // 8]) if k // 8 < len(ipat) else k % 2)
        zero[...] = jnp.zeros(zero.shape, I32)
        b_copy.wait()
        bias[...] = jnp.broadcast_to(bbuf[...].reshape(1, 576).astype(F32), (128, 576)).T
        pruned = []
        for k, copy in enumerate(w_copies):
            copy.wait()
            words = pltpu.bitcast(wbuf[rows * k:rows * (k + 1)], I32)
            pruned += [_prune_packed(words[i:i + 8]) for i in range(0, rows // 2, 8)]
        blocks = {}
        for k in range(3):
            part = pruned[12 * k:12 * k + 8] + 2 * pruned[12 * k + 8:12 * k + 12]
            wt = pltpu.bitcast(jnp.concatenate(part, axis=0), BF16).T.astype(F32)
            for f in range(3):
                blocks[f + 1, k + 1] = wt[192 * f:192 * (f + 1)]
        left = lax.broadcasted_iota(I32, (96, 128), 1) < 64
        forms = _weight_forms(blocks)
        for r, name in enumerate(PRODUCTS):
            a, b = forms[name][:96], forms[name][96:]
            shared = jnp.where(left, a[:, :128], b[:, :128]).astype(BF16)
            lhs[0, r] = shared
            lhs[1, r] = jnp.where(left, a[:, 128:], a[:, :128] - shared.astype(F32)).astype(BF16)
            lhs[2, r] = jnp.where(left, b[:, :128] - shared.astype(F32), b[:, 128:]).astype(BF16)

        def prepare(t, p, k, pin):
            xs, ys = [], []
            for r in (2 * k, 24 + 2 * k, 48 + 2 * k):
                v = [pltpu.bitcast(pin(x_words[9 * t + r // 8, r % 8 + h, p]), BF16).astype(F32) for h in range(2)]
                xs.append(jnp.concatenate([v[0][:8], v[1][:8]], axis=0))
                ys.append(jnp.concatenate([v[0][8:], v[1][8:]], axis=0))
            forms = _input_forms(*xs, *ys)
            for r, name in enumerate(PRODUCTS):
                v = forms[name]
                if r >= 15 // PREP_PARTS:
                    if r % (15 // PREP_PARTS) == 0:
                        yield
                    v = jnp.concatenate([pin(v[:8]), v[8:]], axis=0)
                rhs[p % 2, r, 16 * k:16 * k + 16] = v.astype(BF16)

        def multiply(t, p, jobs, results):
            ring, odd = 9 * (t // 2 % RING), t % 2
            done = len(results)

            def x_rows(r, lo, hi):
                return pltpu.bitcast(rhs_words[p % 2, r, lo // 2:hi // 2], BF16)

            def product(top, s, name):
                n, half = divmod(len(results) - done, 96 // ROWS)
                for job in () if half else jobs.get(n, ()):
                    job()
                r = PRODUCTS.index(name)
                thirds = ((0, 64), (128, 64), (0, 128))[s]
                x = jnp.concatenate([x_rows(r, lo, lo + 64) for lo in thirds], axis=0)
                w = pltpu.bitcast(lhs_words[s, r, top // 2:(top + ROWS) // 2], BF16)
                results.append(jnp.dot(w, x, preferred_element_type=F32))
                return results[-1]

            for top in range(0, 96, ROWS):
                shared = {f: tiles for f, *tiles in
                          _output_blocks(functools.partial(product, top, 0), lambda f, i, v: v)}
                for s in (1, 2):
                    row = lambda f: 192 * f + 96 * (s - 1) + top
                    plus = lambda f, i, v: v + (bias[row(f):row(f) + ROWS] if i == 2 else shared[f][i])
                    for f, first, second in _output_blocks(functools.partial(product, top, s), plus):
                        for k in range(0, ROWS, 8):
                            i, j = divmod((row(f) + k) // 8, 16)
                            at = (ring + i + 4 * odd, j + 8 * odd) if j < 8 else (ring + i + 5 * odd, j - 8 * odd)
                            both = jnp.concatenate([first[k:k + 8], second[k:k + 8]], axis=0)
                            obuf[at + (p,)] = both.astype(BF16)

        wait_quads(0, 0)
        for k in range(12):
            list(prepare(0, 0, k, lambda v: v))

        whole, late, rest = write_plan()
        rows_from = -((READ_AHEAD - 128) // 8)
        assert rows_from + PAIRS * (BATCHES // 2 - 1) <= SWITCH

        def batch(t, carry):
            results = []
            always = zero[t % 2] == 0

            def pin(v):
                if len(results) < PIN_BACK:
                    return v
                recent = results[-PIN_BACK][8 * PIN_ROW:8 * PIN_ROW + 8]
                return jnp.where(always, v, pltpu.bitcast(recent, v.dtype))

            if do_w:
                pl.when((t >= 2 * RING) & (t % 2 == 0))(lambda: wait_written(t // 2 - RING))
            for p in range(PAIRS):
                jobs = {}

                def add(n, when, fn, *args):
                    jobs.setdefault(n, []).append(lambda: pl.when(when)(lambda: fn(*args)))

                for group, (lo, _) in enumerate(QUAD_GROUPS):
                    if p + 1 == 2 * lo:
                        add(0, t < 2, wait_quads, t, group)
                    elif p + 1 == PAIRS and lo == 0:
                        add(0, t == 0, wait_quads, 1, group)
                if p + 1 == PAIRS:
                    add(0, (t % 2 == 1) & (t < BATCHES - 1), wait_rows, t + 1, 144)
                if p + 1 == PAIRS // 2:
                    add(0, (t % 2 == 0) & (t >= 2) & (t < BATCHES - (2 if READ_OVERLAP else 0)), wait_rows, t + 1, 144)
                    if READ_OVERLAP:
                        add(0, t == BATCHES - 2, wait_rows, 0, READ_OVERLAP)
                if p == SWITCH % PAIRS and do_w:
                    add(0, t == SWITCH // PAIRS, wait_rows, BATCHES - 1, 144 - READ_OVERLAP)
                    for k in range(WRITE_AHEAD):
                        add(0, t == SWITCH // PAIRS, write, 0, 0, 9, k // 4, k % 4)
                at = lambda i, n: (DMA_AT + PASSES * i // n) % PASSES
                for i in range(8):
                    k = READ_AHEAD + 8 * p + i
                    if k < 128:
                        add(at(i, 8), t == 0, read_quad, k, k % 2)
                d = t + (p >= rows_from)
                for i in range(18):
                    add(at(i, 18), (d >= 1) & (d < BATCHES // 2), read_row, d, (p - rows_from) % PAIRS * 18 + i)
                for i in range(8 if do_w else 0):
                    if i % 2 == 0:
                        ahead, k = divmod(4 * (p - SWITCH) + WRITE_AHEAD + i // 2, 64)
                        add(at(i, 8), (PAIRS * t + p >= SWITCH) & (t + ahead < whole),
                            write, t + ahead, 0, 9, k // 4, k % 4)
                    for when, copy in late.get((p, i), ()):
                        add(at(i, 8), t == when, write, *copy)
                following = (t, p + 1) if p + 1 < PAIRS else (jnp.minimum(t + 1, BATCHES - 1), 0)
                for k in range(12):
                    parts = prepare(*following, k, pin)
                    for i in range(PREP_PARTS):
                        jobs.setdefault(int(PREP_AT + PREP_EVERY * k) + PART_EVERY * i, []).append(
                            functools.partial(next, parts, None))
                assert max(jobs) < PASSES
                multiply(t, p, jobs, results)
            return carry

        lax.fori_loop(0, BATCHES, batch, 0)
        if do_w:
            for copy in rest:
                write(*copy)
            for d in range(BATCHES // 2 - RING, BATCHES // 2):
                wait_written(d)
        else:
            write(0, 0, 1, 0, 0)
            pltpu.make_async_copy(obuf.at[0, 0, pl.ds(0, 4)], obuf.at[0, 0, pl.ds(0, 4)], osem.at[0]).wait()

    def fn(x, w, b):
        assert x.shape == (16, 4096, 576) and w.shape == (576, 576)
        tiles = x.reshape(16, 32, 128, 72, 8).transpose(0, 3, 1, 4, 2)
        out = pl.pallas_call(
            _kernel,
            in_specs=[pl.BlockSpec(memory_space=pl.ANY)] * 3,
            out_specs=pl.BlockSpec(memory_space=pl.ANY),
            out_shape=jax.ShapeDtypeStruct((72, 16, 16, 16, 128), x.dtype),
            scratch_shapes=[
                pltpu.VMEM((144, 8, 16, 16, 128), BF16),
                pltpu.VMEM((9 * RING, 16, 16, 16, 128), BF16),
                pltpu.VMEM((576, 576), BF16),
                pltpu.VMEM((576,), BF16),
                pltpu.VMEM((3, 15, 96, 128), BF16),
                pltpu.VMEM((2, 15, 192, 128), BF16),
                pltpu.VMEM((576, 128), F32),
                pltpu.VMEM((2, 8, 128), I32),
                pltpu.SemaphoreType.DMA((3, len(QUAD_GROUPS))),
                pltpu.SemaphoreType.DMA((16,)),
                pltpu.SemaphoreType.DMA((8,)),
            ],
            compiler_params=pltpu.CompilerParams(
                vmem_limit_bytes=127 * 1024 * 1024,
                flags={"XLA_TPU_RESCHEDULE_DMA_DONES": True},
                disable_bounds_checks=True,
                disable_semaphore_checks=True,
            ),
        )(tiles.reshape(144, 8, 16, 16, 128), w, b)
        return out.reshape(16, 72, 32, 8, 128).transpose(0, 2, 4, 1, 3).reshape(x.shape)
    return fn


@jax.jit
def pallas_standalone__structured_sparse_n_m__ragged_kernel(x, w, b):
    return make(READ_OVERLAP=40, WPARTS=1)(x, w, b)
```

```python
import functools

import jax
import jax.numpy as jnp
from jax import lax
import jax.experimental.pallas as pl
import jax.experimental.pallas.tpu as pltpu

F32, BF16, I32 = jnp.float32, jnp.bfloat16, jnp.int32

PRODUCTS = ("r1", "v1", "v2", "v3", "u3", "u1", "u2", "q1", "p2", "r2", "w1", "w3", "w2", "p3", "q3")


def _weight_forms(a):
    return dict(
        r1=a[1, 1] + a[1, 2] - a[3, 1], q1=a[1, 1] - a[2, 1] + a[1, 3],
        r2=a[2, 2] + a[2, 1] - a[3, 2], p2=a[2, 2] - a[1, 2] + a[2, 3],
        p3=a[3, 3] - a[1, 3] + a[3, 2], q3=a[3, 3] + a[3, 1] - a[2, 3],
        u1=a[2, 1] + a[1, 2], u2=a[2, 1], u3=a[1, 2],
        v1=a[3, 1] + a[1, 3], v2=a[3, 1], v3=a[1, 3],
        w1=a[2, 3] + a[3, 2], w2=a[2, 3], w3=a[3, 2])


def _input_forms(x1, x2, x3, y1, y2, y3):
    s1, s2, s3 = x1 - y1, x2 - y2, x3 - y3
    return dict(r1=x1, q1=s1, r2=y2, p2=s2, p3=x3, q3=y3,
                u1=x1 - y2, u2=y2 - y1, u3=x2 - x1,
                v1=s1 + y3, v2=y1 - y3, v3=s3 - s1,
                w1=s2 - x3, w2=s3 - s2, w3=x3 - x2)


def _output_blocks(prod, plus):
    r1, v1, v2, v3 = prod("r1"), prod("v1"), prod("v2"), prod("v3")
    both1 = plus(0, 2, r1) + v1 + v2
    first3 = plus(2, 0, v1) + v3
    first1 = plus(0, 0, v3) + both1
    u3, u1, u2, q1 = prod("u3"), prod("u1"), prod("u2"), prod("q1")
    first2 = plus(1, 0, u3) + u1
    yield 0, first1 + u3, (plus(0, 1, both1) - q1) - (u1 + u2)
    p2, r2, w1, w3 = prod("p2"), prod("r2"), prod("w1"), prod("w3")
    both2 = plus(1, 2, r2) - w1 - w3
    first2 = (first2 + p2) + both2
    second2 = plus(1, 1, both2) - u2
    both3 = plus(2, 2, v2) - w3
    second3 = plus(2, 1, both3) - w1
    first3 = first3 + both3
    w2 = prod("w2")
    yield 1, first2, second2 - w2
    second3 = second3 - w2
    p3, q3 = prod("p3"), prod("q3")
    yield 2, first3 + p3, second3 + q3


def _prune_packed(u):
    mate = lax.broadcasted_iota(I32, u.shape, 0) ^ 1
    lo = pltpu.bitcast((u << 16) & 0x7FFFFFFF, F32)
    hi = pltpu.bitcast(u & 0x7FFF0000, F32)
    big, small = jnp.maximum(lo, hi), jnp.minimum(lo, hi)
    nbig = jnp.take_along_axis(big, mate, axis=0, mode="promise_in_bounds")
    nsmall = jnp.take_along_axis(small, mate, axis=0, mode="promise_in_bounds")
    thr = jnp.maximum(jnp.minimum(big, nbig), jnp.maximum(small, nsmall))
    return u & (jnp.where(lo < thr, 0, 0xFFFF) | jnp.where(hi < thr, 0, -65536))


def make(do_w=True, RING=5, READ_AHEAD=36, SWITCH=123, READ_OVERLAP=32, WRITE_AHEAD=4, TAIL=(2, 1, 1),
         PREP_AT=2, PREP_EVERY=3.0, PIN_BACK=5, PIN_ROW=1, PREP_PARTS=5, PART_EVERY=1, DMA_AT=0,
         ipat="001", WPARTS=1, late_rate=8, rowstep=16, skew=0, lo_first=1, probe=0, do_c=True, delay=16):
    BATCHES, PAIRS, PASSES, ROWS = 16, 16, 45, 48
    QUAD_GROUPS = ((0, 1), (1, 2), (2, 4))
    if not do_w:
        READ_OVERLAP = 0

    def write_plan():
        whole = 0
        while whole < BATCHES // 2 - 1 and SWITCH + (64 * whole - WRITE_AHEAD) // 4 >= 2 * PAIRS * (whole + 1):
            whole += 1
        todo, pos = [], 8 * whole
        for n in [4] * ((4 * BATCHES - pos - sum(TAIL)) // 4) + list(TAIL):
            t, c0 = divmod(pos, 4)
            assert c0 + n <= 4
            for r in range(16):
                i, j = divmod(72 * (t % 2) + r, 16)
                todo += [(PAIRS * t + 4 * (c0 + n), (t // 2, i, len(range(r, 72, 16)), j, c))
                         for c in range(c0, c0 + n)]
            pos += n
        assert pos == 4 * BATCHES
        late = {}
        for step in range(SWITCH - (WRITE_AHEAD - 64 * whole) // 4, BATCHES * PAIRS):
            for slot in range(late_rate):
                if todo and todo[0][0] <= step:
                    late.setdefault((step % PAIRS, slot * 8 // late_rate), []).append((step // PAIRS, todo.pop(0)[1]))
        return whole, late, [copy for _, copy in todo]

    def _kernel(x_hbm, w_hbm, b_hbm, o_hbm, xbuf, obuf, wbuf, bbuf, lhs, rhs, bias, zero,
                qsem, xsem, osem):
        x_words, lhs_words, rhs_words = xbuf.bitcast(I32), lhs.bitcast(I32), rhs.bitcast(I32)

        def read(k, sem, *at):
            pltpu.make_async_copy(x_hbm.at[at], xbuf.at[at], sem).start(priority=(k + lo_first) % 2)

        def read_quad(k):
            c, j = divmod(k, 8)
            group = next(g for g, (lo, hi) in enumerate(QUAD_GROUPS) if lo <= c < hi)
            read(k, qsem.at[group], pl.ds(0, 9), j, pl.ds(2 * c, 2))

        def read_half(k):
            half, r = divmod(72 + k, 72)
            row = 72 * (half // 2) + (r % 18 * 20 + r // 18) % 72
            read(k, xsem.at[half], row // 8, row % 8, pl.ds(8 * (half % 2), 8))

        def read_sweep(d, k):
            j, m = divmod(k, 36)
            i = jnp.where(d == 1, 18 + 2 * (m % 9) + m // 9 % 2, 36 * (d // 2) + m)
            h = jnp.where(d == 1, m // 18, d % 2)
            sem = 3 + d
            if k >= 288 - READ_OVERLAP:
                sem = jnp.where(d == 7, 0, sem)
            read(k, xsem.at[sem], i, j, pl.ds(8 * h, 8))

        def wait_read(sem, *at):
            pltpu.make_async_copy(xbuf.at[at], xbuf.at[at], sem).wait()

        def wait_quads(group):
            lo, hi = QUAD_GROUPS[group]
            wait_read(qsem.at[group], pl.ds(0, 9), slice(None), pl.ds(0, 2 * (hi - lo)))

        def wait_rows(sem, n):
            assert n % 2 == 0
            wait_read(xsem.at[sem], pl.ds(0, n // 2), pl.ds(0, 2), pl.ds(0, 8))

        def write(d, i, n, j, c):
            pltpu.make_async_copy(obuf.at[pl.ds(9 * (d % RING) + i, n), j, pl.ds(4 * c, 4)],
                                  o_hbm.at[pl.ds(9 * d + i, n), j, pl.ds(4 * c, 4)], osem.at[d]).start()

        def wait_written(d):
            pltpu.make_async_copy(obuf.at[pl.ds(0, 9)], obuf.at[pl.ds(0, 9)], osem.at[d]).wait()

        rows = 576 // WPARTS
        w_copies = [pltpu.make_async_copy(w_hbm.at[pl.ds(rows * k, rows)], wbuf.at[pl.ds(rows * k, rows)],
                                          qsem.at[4]) for k in range(WPARTS)]
        b_copy = pltpu.make_async_copy(b_hbm, bbuf, qsem.at[3])
        b_copy.start()
        for k, copy in enumerate(w_copies):
            copy.start(priority=(k + lo_first + WPARTS) % 2)
        for k in range(32):
            read_quad(k)
        for k in range(READ_AHEAD):
            read_half(k)
        zero[...] = jnp.zeros(zero.shape, I32)
        b_copy.wait()
        bias[...] = jnp.broadcast_to(bbuf[...].reshape(1, 576).astype(F32), (128, 576)).T
        for copy in w_copies:
            copy.wait()
        words = pltpu.bitcast(wbuf[...], I32)
        pruned = [_prune_packed(words[i:i + 8]) for i in range(0, 288, 8)]
        blocks = {}
        for k in range(3):
            part = pruned[12 * k:12 * k + 8] + 2 * pruned[12 * k + 8:12 * k + 12]
            wt = pltpu.bitcast(jnp.concatenate(part, axis=0), BF16).T.astype(F32)
            for f in range(3):
                blocks[f + 1, k + 1] = wt[192 * f:192 * (f + 1)]
        left = lax.broadcasted_iota(I32, (96, 128), 1) < 64
        forms = _weight_forms(blocks)
        for r, name in enumerate(PRODUCTS):
            a, b = forms[name][:96], forms[name][96:]
            shared = jnp.where(left, a[:, :128], b[:, :128]).astype(BF16)
            lhs[0, r] = shared
            lhs[1, r] = jnp.where(left, a[:, 128:], a[:, :128] - shared.astype(F32)).astype(BF16)
            lhs[2, r] = jnp.where(left, b[:, :128] - shared.astype(F32), b[:, 128:]).astype(BF16)

        def prepare(t, p, k, pin):
            xs, ys = [], []
            for r in (2 * k, 24 + 2 * k, 48 + 2 * k):
                v = [pltpu.bitcast(pin(x_words[9 * t + r // 8, r % 8 + h, p]), BF16).astype(F32) for h in range(2)]
                xs.append(jnp.concatenate([v[0][:8], v[1][:8]], axis=0))
                ys.append(jnp.concatenate([v[0][8:], v[1][8:]], axis=0))
            forms = _input_forms(*xs, *ys)
            for r, name in enumerate(PRODUCTS):
                v = forms[name]
                if r >= 15 // PREP_PARTS:
                    if r % (15 // PREP_PARTS) == 0:
                        yield
                    v = jnp.concatenate([pin(v[:8]), v[8:]], axis=0)
                rhs[p % 2, r, 16 * k:16 * k + 16] = v.astype(BF16)

        def multiply(t, p, jobs, results):
            ring, odd = 9 * (t // 2 % RING), t % 2
            done = len(results)

            def x_rows(r, lo, hi):
                return pltpu.bitcast(rhs_words[p % 2, r, lo // 2:hi // 2], BF16)

            def product(top, s, name):
                n, half = divmod(len(results) - done, 96 // ROWS)
                for job in () if half else jobs.get(n, ()):
                    job()
                r = PRODUCTS.index(name)
                thirds = ((0, 64), (128, 64), (0, 128))[s]
                x = jnp.concatenate([x_rows(r, lo, lo + 64) for lo in thirds], axis=0)
                w = pltpu.bitcast(lhs_words[s, r, top // 2:(top + ROWS) // 2], BF16)
                results.append(jnp.dot(w, x, preferred_element_type=F32))
                return results[-1]

            for top in range(0, 96, ROWS):
                shared = {f: tiles for f, *tiles in
                          _output_blocks(functools.partial(product, top, 0), lambda f, i, v: v)}
                for s in (1, 2):
                    row = lambda f: 192 * f + 96 * (s - 1) + top
                    plus = lambda f, i, v: v + (bias[row(f):row(f) + ROWS] if i == 2 else shared[f][i])
                    for f, first, second in _output_blocks(functools.partial(product, top, s), plus):
                        for k in range(0, ROWS, 8):
                            i, j = divmod((row(f) + k) // 8, 16)
                            at = (ring + i + 4 * odd, j + 8 * odd) if j < 8 else (ring + i + 5 * odd, j - 8 * odd)
                            both = jnp.concatenate([first[k:k + 8], second[k:k + 8]], axis=0)
                            obuf[at + (p,)] = both.astype(BF16)

        wait_quads(0)
        for k in range(12):
            list(prepare(0, 0, k, lambda v: v))

        whole, late, rest = write_plan()
        first = 216 - READ_AHEAD
        assert first + 7 * 288 <= 18 * SWITCH

        def batch(t, carry):
            results = []
            always = zero[t % 2] == 0

            def pin(v):
                if len(results) < PIN_BACK:
                    return v
                recent = results[-PIN_BACK][8 * PIN_ROW:8 * PIN_ROW + 8]
                return jnp.where(always, v, pltpu.bitcast(recent, v.dtype))

            if do_w:
                pl.when((t >= 2 * RING) & (t % 2 == 0))(lambda: wait_written(t // 2 - RING))
            for p in range(PAIRS):
                jobs = {}

                def add(n, when, fn, *args):
                    jobs.setdefault(n, []).append(lambda: pl.when(when)(lambda: fn(*args)))

                for group, (lo, _) in enumerate(QUAD_GROUPS):
                    if p + 1 == 2 * lo:
                        add(0, t == 0, wait_quads, group)
                if p + 1 == PAIRS // 2:
                    add(0, t < 2, wait_rows, 2 * t + 1, 72)
                    add(0, (t == 4) | (t == 8), wait_rows, 4 + t // 2, 288)
                    add(0, t == 12, wait_rows, *((0, READ_OVERLAP) if READ_OVERLAP else (10, 288)))
                if p + 1 == PAIRS:
                    add(0, t == 0, wait_rows, 2, 72)
                    add(0, (t == 1) | ((t % 4 == 3) & (t < BATCHES - 1)), wait_rows, 4 + t // 2, 288)
                if p == SWITCH % PAIRS and do_w:
                    add(0, t == SWITCH // PAIRS, wait_rows, 10, 288 - READ_OVERLAP)
                    for k in range(WRITE_AHEAD):
                        add(0, t == SWITCH // PAIRS, write, 0, 0, 9, k // 4, k % 4)
                at = lambda i, n: (DMA_AT + PASSES * i // n) % PASSES
                for i in range(18):
                    slot = 18 * p + i
                    d = t + 1
                    if slot < first:
                        d = t
                        add(at(i, 18), t == 0, read_half, READ_AHEAD + slot)
                    add(at(i, 18), (d >= 1) & (d <= 7), read_sweep, d, (slot - first) % 288)
                for i in range(8 if do_w else 0):
                    if i % 2 == 0:
                        ahead, k = divmod(4 * (p - SWITCH) + WRITE_AHEAD + i // 2, 64)
                        add(at(i, 8), (PAIRS * t + p >= SWITCH) & (t + ahead < whole),
                            write, t + ahead, 0, 9, k // 4, k % 4)
                    for when, copy in late.get((p, i), ()):
                        add(at(i, 8), t == when, write, *copy)
                following = (t, p + 1) if p + 1 < PAIRS else (jnp.minimum(t + 1, BATCHES - 1), 0)
                for k in range(12):
                    parts = prepare(*following, k, pin)
                    for i in range(PREP_PARTS):
                        jobs.setdefault(int(PREP_AT + PREP_EVERY * k) + PART_EVERY * i, []).append(
                            functools.partial(next, parts, None))
                assert max(jobs) < PASSES
                if do_c:
                    multiply(t, p, jobs, results)
                else:
                    for n in range(PASSES):
                        for job in jobs.get(n, ()):
                            if not isinstance(job, functools.partial):
                                job()
                        pl.delay(delay)
            return carry

        if probe:
            lax.fori_loop(0, 7, batch, 0)
            for k in range(288 - first, 288):
                read_sweep(7, k)
                pl.delay(36)
            for sem in range(7, 11):
                wait_rows(sem, 288)
            if probe == 2:
                return
            write(0, 0, 1, 0, 0)
            pltpu.make_async_copy(obuf.at[0, 0, pl.ds(0, 4)], obuf.at[0, 0, pl.ds(0, 4)], osem.at[0]).wait()
            return
        lax.fori_loop(0, BATCHES, batch, 0)
        if do_w:
            for copy in rest:
                write(*copy)
            for d in range(BATCHES // 2 - RING, BATCHES // 2):
                wait_written(d)
        else:
            write(0, 0, 1, 0, 0)
            pltpu.make_async_copy(obuf.at[0, 0, pl.ds(0, 4)], obuf.at[0, 0, pl.ds(0, 4)], osem.at[0]).wait()

    def fn(x, w, b):
        assert x.shape == (16, 4096, 576) and w.shape == (576, 576)
        tiles = x.reshape(16, 32, 128, 72, 8).transpose(0, 3, 1, 4, 2)
        out = pl.pallas_call(
            _kernel,
            in_specs=[pl.BlockSpec(memory_space=pl.ANY)] * 3,
            out_specs=pl.BlockSpec(memory_space=pl.ANY),
            out_shape=jax.ShapeDtypeStruct((72, 16, 16, 16, 128), x.dtype),
            scratch_shapes=[
                pltpu.VMEM((144, 8, 16, 16, 128), BF16),
                pltpu.VMEM((9 * RING, 16, 16, 16, 128), BF16),
                pltpu.VMEM((576, 576), BF16),
                pltpu.VMEM((576,), BF16),
                pltpu.VMEM((3, 15, 96, 128), BF16),
                pltpu.VMEM((2, 15, 192, 128), BF16),
                pltpu.VMEM((576, 128), F32),
                pltpu.VMEM((2, 8, 128), I32),
                pltpu.SemaphoreType.DMA((5,)),
                pltpu.SemaphoreType.DMA((11,)),
                pltpu.SemaphoreType.DMA((8,)),
            ],
            compiler_params=pltpu.CompilerParams(
                vmem_limit_bytes=127 * 1024 * 1024,
                flags={"XLA_TPU_RESCHEDULE_DMA_DONES": True},
                disable_bounds_checks=True,
                disable_semaphore_checks=True,
            ),
        )(tiles.reshape(144, 8, 16, 16, 128), w, b)
        return out.reshape(16, 72, 32, 8, 128).transpose(0, 2, 4, 1, 3).reshape(x.shape)
    return fn


@jax.jit
def pallas_standalone__structured_sparse_n_m__ragged_kernel(x, w, b):
    return make()(x, w, b)
```

```python
import functools

import jax
import jax.numpy as jnp
from jax import lax
import jax.experimental.pallas as pl
import jax.experimental.pallas.tpu as pltpu

F32, BF16, I32 = jnp.float32, jnp.bfloat16, jnp.int32

BATCHES = 16
PAIRS = 16
PASSES = 45
ROWS = 48
RING = 5
READ_AHEAD = 36
SWITCH = 124
WRITE_AHEAD = 4
TAIL = (8, 4, 3, 1)
QUADS = ((0, 1), (1, 2), (2, 4))
PREP_AT, PREP_EVERY, PREP_PARTS, PIN_BACK, PIN_ROW = 2, 3, 5, 5, 1

PRODUCTS = ("r1", "v1", "v2", "v3", "u3", "u1", "u2", "q1", "p2", "r2", "w1", "w3", "w2", "p3", "q3")


def _weight_forms(a):
    return dict(
        r1=a[1, 1] + a[1, 2] - a[3, 1], q1=a[1, 1] - a[2, 1] + a[1, 3],
        r2=a[2, 2] + a[2, 1] - a[3, 2], p2=a[2, 2] - a[1, 2] + a[2, 3],
        p3=a[3, 3] - a[1, 3] + a[3, 2], q3=a[3, 3] + a[3, 1] - a[2, 3],
        u1=a[2, 1] + a[1, 2], u2=a[2, 1], u3=a[1, 2],
        v1=a[3, 1] + a[1, 3], v2=a[3, 1], v3=a[1, 3],
        w1=a[2, 3] + a[3, 2], w2=a[2, 3], w3=a[3, 2])


def _input_forms(x1, x2, x3, y1, y2, y3):
    s1, s2, s3 = x1 - y1, x2 - y2, x3 - y3
    return dict(r1=x1, q1=s1, r2=y2, p2=s2, p3=x3, q3=y3,
                u1=x1 - y2, u2=y2 - y1, u3=x2 - x1,
                v1=s1 + y3, v2=y1 - y3, v3=s3 - s1,
                w1=s2 - x3, w2=s3 - s2, w3=x3 - x2)


def _output_blocks(prod, plus):
    r1, v1, v2, v3 = prod("r1"), prod("v1"), prod("v2"), prod("v3")
    both1 = plus(0, 2, r1) + v1 + v2
    first3 = plus(2, 0, v1) + v3
    first1 = plus(0, 0, v3) + both1
    u3, u1, u2, q1 = prod("u3"), prod("u1"), prod("u2"), prod("q1")
    first2 = plus(1, 0, u3) + u1
    yield 0, first1 + u3, (plus(0, 1, both1) - q1) - (u1 + u2)
    p2, r2, w1, w3 = prod("p2"), prod("r2"), prod("w1"), prod("w3")
    both2 = plus(1, 2, r2) - w1 - w3
    first2 = (first2 + p2) + both2
    second2 = plus(1, 1, both2) - u2
    both3 = plus(2, 2, v2) - w3
    second3 = plus(2, 1, both3) - w1
    first3 = first3 + both3
    w2 = prod("w2")
    yield 1, first2, second2 - w2
    second3 = second3 - w2
    p3, q3 = prod("p3"), prod("q3")
    yield 2, first3 + p3, second3 + q3


def _prune_packed(u):
    mate = lax.broadcasted_iota(I32, u.shape, 0) ^ 1
    lo = pltpu.bitcast((u << 16) & 0x7FFFFFFF, F32)
    hi = pltpu.bitcast(u & 0x7FFF0000, F32)
    big, small = jnp.maximum(lo, hi), jnp.minimum(lo, hi)
    nbig = jnp.take_along_axis(big, mate, axis=0, mode="promise_in_bounds")
    nsmall = jnp.take_along_axis(small, mate, axis=0, mode="promise_in_bounds")
    thr = jnp.maximum(jnp.minimum(big, nbig), jnp.maximum(small, nsmall))
    return u & (jnp.where(lo < thr, 0, 0xFFFF) | jnp.where(hi < thr, 0, -65536))


def _write_plan():
    whole, left = divmod(4 * BATCHES - sum(TAIL), 8)
    assert not left and SWITCH + (64 * (whole - 1) - WRITE_AHEAD) // 4 >= 2 * PAIRS * whole
    todo, pos = [], 8 * whole
    for n in TAIL:
        t, c0 = divmod(pos, 4)
        assert c0 + n <= 4 or (n == 8 and pos % 8 == 0)
        pos += n
        for r in range(16):
            i, j = divmod(72 * (t % 2) + r, 16)
            tiles = len(range(r, 144 if n == 8 else 72, 16))
            todo += [(4 * pos, (t // 2, i, tiles, j, c)) for c in range(c0, min(c0 + n, 4))]
    late = {}
    for step in range(SWITCH - (WRITE_AHEAD - 64 * whole) // 4, BATCHES * PAIRS):
        for slot in range(8):
            if todo and todo[0][0] <= step:
                late.setdefault((step % PAIRS, slot), []).append((step // PAIRS, todo.pop(0)[1]))
    return whole, late, [copy for _, copy in todo]


def _kernel(x_hbm, w_hbm, b_hbm, o_hbm, xbuf, obuf, wbuf, bbuf, lhs, rhs, bias, zero,
            first_sem, x_sem, o_sem):
    x_words, lhs_words, rhs_words = xbuf.bitcast(I32), lhs.bitcast(I32), rhs.bitcast(I32)
    every = slice(None)

    def x_copy(sem, *at):
        return pltpu.make_async_copy(x_hbm.at[at], xbuf.at[at], sem)

    def read_quad(k):
        c, j = divmod(k, 8)
        group = next(g for g, (lo, hi) in enumerate(QUADS) if lo <= c < hi)
        x_copy(first_sem.at[group], pl.ds(0, 9), j, pl.ds(2 * c, 2)).start(priority=1 - k % 2)

    def wait_quads(group):
        lo, hi = QUADS[group]
        x_copy(first_sem.at[group], pl.ds(0, 9), every, pl.ds(2 * lo, 2 * (hi - lo))).wait()

    def read_half(k):
        half, r = divmod(72 + k, 72)
        i, j = divmod(72 * (half // 2) + (r % 18 * 20 + r // 18) % 72, 8)
        x_copy(x_sem.at[half], i, j, pl.ds(8 * (half % 2), 8)).start(priority=1 - k % 2)

    def wait_half(half):
        x_copy(x_sem.at[half], pl.ds(9 * (half // 2), 9), every, pl.ds(8 * (half % 2), 8)).wait()

    def read_sweep(d, k):
        j, m = divmod(k, 36)
        i = jnp.where(d == 1, 18 + 2 * (m % 9) + m // 9 % 2, 36 * (d // 2) + m)
        half = jnp.where(d == 1, m // 18, d % 2)
        sem = jnp.where(d == 7, 0, 3 + d) if j == 7 else 3 + d
        x_copy(x_sem.at[sem], i, j, pl.ds(8 * half, 8)).start(priority=1 - k % 2)

    def wait_sweep(d, sem, j=every):
        x_copy(x_sem.at[sem], pl.ds(36 * (d // 2), 36), j, pl.ds(8 * (d % 2), 8)).wait()

    def o_copy(d, i, n, *at):
        return pltpu.make_async_copy(obuf.at[(pl.ds(9 * (d % RING) + i, n), *at)],
                                     o_hbm.at[(pl.ds(9 * d + i, n), *at)], o_sem.at[d])

    def write(d, i, n, j, c):
        o_copy(d, i, n, j, pl.ds(4 * c, 4)).start()

    b_copy = pltpu.make_async_copy(b_hbm, bbuf, first_sem.at[3])
    w_copy = pltpu.make_async_copy(w_hbm, wbuf, first_sem.at[4])
    b_copy.start()
    w_copy.start()
    for k in range(32):
        read_quad(k)
    for k in range(READ_AHEAD):
        read_half(k)
    zero[...] = jnp.zeros(zero.shape, I32)
    b_copy.wait()
    bias[...] = jnp.broadcast_to(bbuf[...].reshape(1, 576).astype(F32), (128, 576)).T
    w_copy.wait()
    words = pltpu.bitcast(wbuf[...], I32)
    pruned = [_prune_packed(words[i:i + 8]) for i in range(0, 288, 8)]
    blocks = {}
    for k in range(3):
        part = pruned[12 * k:12 * k + 8] + 2 * pruned[12 * k + 8:12 * k + 12]
        wt = pltpu.bitcast(jnp.concatenate(part, axis=0), BF16).T.astype(F32)
        for f in range(3):
            blocks[f + 1, k + 1] = wt[192 * f:192 * (f + 1)]
    left = lax.broadcasted_iota(I32, (96, 128), 1) < 64
    forms = _weight_forms(blocks)
    for r, name in enumerate(PRODUCTS):
        a, b = forms[name][:96], forms[name][96:]
        shared = jnp.where(left, a[:, :128], b[:, :128]).astype(BF16)
        lhs[0, r] = shared
        lhs[1, r] = jnp.where(left, a[:, 128:], a[:, :128] - shared.astype(F32)).astype(BF16)
        lhs[2, r] = jnp.where(left, b[:, :128] - shared.astype(F32), b[:, 128:]).astype(BF16)

    def prepare(t, p, k, pin):
        xs, ys = [], []
        for r in (2 * k, 24 + 2 * k, 48 + 2 * k):
            v = [pltpu.bitcast(pin(x_words[9 * t + r // 8, r % 8 + h, p]), BF16).astype(F32)
                 for h in range(2)]
            xs.append(jnp.concatenate([v[0][:8], v[1][:8]], axis=0))
            ys.append(jnp.concatenate([v[0][8:], v[1][8:]], axis=0))
        forms = _input_forms(*xs, *ys)
        for r, name in enumerate(PRODUCTS):
            v = forms[name]
            if r >= 15 // PREP_PARTS:
                if r % (15 // PREP_PARTS) == 0:
                    yield
                v = jnp.concatenate([pin(v[:8]), v[8:]], axis=0)
            rhs[p % 2, r, 16 * k:16 * k + 16] = v.astype(BF16)

    def multiply(t, p, jobs, results):
        slot, odd = 9 * (t // 2 % RING), t % 2
        done = len(results)

        def product(top, s, name):
            n, part = divmod(len(results) - done, 96 // ROWS)
            for job in () if part else jobs.get(n, ()):
                job()
            r = PRODUCTS.index(name)
            x = jnp.concatenate([pltpu.bitcast(rhs_words[p % 2, r, 32 * c:32 * c + 32], BF16)
                                 for c in ((0, 1), (2, 1), (0, 2))[s]], axis=0)
            w = pltpu.bitcast(lhs_words[s, r, top // 2:(top + ROWS) // 2], BF16)
            results.append(jnp.dot(w, x, preferred_element_type=F32))
            return results[-1]

        for top in range(0, 96, ROWS):
            shared = {f: tiles for f, *tiles in
                      _output_blocks(functools.partial(product, top, 0), lambda f, i, v: v)}
            for s in (1, 2):
                row = lambda f: 192 * f + 96 * (s - 1) + top
                plus = lambda f, i, v: v + (bias[row(f):row(f) + ROWS] if i == 2 else shared[f][i])
                for f, first, second in _output_blocks(functools.partial(product, top, s), plus):
                    for k in range(0, ROWS, 8):
                        i, j = divmod((row(f) + k) // 8, 16)
                        if j < 8:
                            at = (slot + i + 4 * odd, j + 8 * odd, p)
                        else:
                            at = (slot + i + 5 * odd, j - 8 * odd, p)
                        both = jnp.concatenate([first[k:k + 8], second[k:k + 8]], axis=0)
                        obuf[at] = both.astype(BF16)

    wait_quads(0)
    for k in range(12):
        list(prepare(0, 0, k, lambda v: v))

    whole, late, rest = _write_plan()
    sweeps_from = 216 - READ_AHEAD
    assert sweeps_from + 7 * 288 <= 18 * SWITCH < 18 * PAIRS * 2 * RING

    def batch(t, carry):
        results = []
        always = zero[t % 2] == 0

        def pin(v):
            if len(results) < PIN_BACK:
                return v
            recent = results[-PIN_BACK][8 * PIN_ROW:8 * PIN_ROW + 8]
            return jnp.where(always, v, pltpu.bitcast(recent, v.dtype))

        pl.when((t >= 2 * RING) & (t % 2 == 0))(lambda: o_copy(t // 2 - RING, 0, 9).wait())
        for p in range(PAIRS):
            jobs = {}

            def add(n, when, fn, *args):
                jobs.setdefault(n, []).append(lambda: pl.when(when)(lambda: fn(*args)))

            for group, (lo, _) in enumerate(QUADS):
                if p + 1 == 2 * lo:
                    add(0, t == 0, wait_quads, group)
            if p + 1 == PAIRS // 2:
                add(0, t < 2, wait_half, 2 * t + 1)
                add(0, (t == 4) | (t == 8), wait_sweep, t // 2 + 1, t // 2 + 4)
                add(0, t == 12, wait_sweep, 7, 0, 7)
            if p + 1 == PAIRS:
                add(0, t == 0, wait_half, 2)
                add(0, t == 1, lambda: x_copy(x_sem.at[4], pl.ds(18, 18)).wait())
                add(0, (t % 4 == 3) & (t < BATCHES - 1), wait_sweep, t // 2 + 1, t // 2 + 4)
            if p == SWITCH % PAIRS:
                add(0, t == SWITCH // PAIRS, wait_sweep, 7, 10, pl.ds(0, 7))
                for k in range(WRITE_AHEAD):
                    add(0, t == SWITCH // PAIRS, write, 0, 0, 9, k // 4, k % 4)
            for i in range(18):
                k, d = 18 * p + i, t + 1
                if k < sweeps_from:
                    d = t
                    add(PASSES * i // 18, t == 0, read_half, READ_AHEAD + k)
                add(PASSES * i // 18, (d >= 1) & (d <= 7), read_sweep, d, (k - sweeps_from) % 288)
            for i in range(8):
                if i % 2 == 0:
                    ahead, k = divmod(4 * (p - SWITCH) + WRITE_AHEAD + i // 2, 64)
                    add(PASSES * i // 8, (PAIRS * t + p >= SWITCH) & (t + ahead < whole),
                        write, t + ahead, 0, 9, k // 4, k % 4)
                for when, copy in late.get((p, i), ()):
                    add(PASSES * i // 8, t == when, write, *copy)
            following = (t, p + 1) if p + 1 < PAIRS else (jnp.minimum(t + 1, BATCHES - 1), 0)
            for k in range(12):
                parts = prepare(*following, k, pin)
                for i in range(PREP_PARTS):
                    jobs.setdefault(PREP_AT + PREP_EVERY * k + i, []).append(
                        functools.partial(next, parts, None))
            assert max(jobs) < PASSES
            multiply(t, p, jobs, results)
        return carry

    lax.fori_loop(0, BATCHES, batch, 0)
    for copy in rest:
        write(*copy)
    for d in range(BATCHES // 2 - RING, BATCHES // 2):
        o_copy(d, 0, 9).wait()


@jax.jit
def pallas_standalone__structured_sparse_n_m__ragged_kernel(
    x: jax.Array,
    w: jax.Array,
    b: jax.Array,
):
    assert x.shape == (16, 4096, 576) and w.shape == (576, 576)
    tiles = x.reshape(16, 32, 128, 72, 8).transpose(0, 3, 1, 4, 2)
    out = pl.pallas_call(
        _kernel,
        in_specs=[pl.BlockSpec(memory_space=pl.ANY)] * 3,
        out_specs=pl.BlockSpec(memory_space=pl.ANY),
        out_shape=jax.ShapeDtypeStruct((72, 16, PAIRS, 16, 128), x.dtype),
        scratch_shapes=[
            pltpu.VMEM((144, 8, PAIRS, 16, 128), BF16),
            pltpu.VMEM((9 * RING, 16, PAIRS, 16, 128), BF16),
            pltpu.VMEM((576, 576), BF16),
            pltpu.VMEM((576,), BF16),
            pltpu.VMEM((3, 15, 96, 128), BF16),
            pltpu.VMEM((2, 15, 192, 128), BF16),
            pltpu.VMEM((576, 128), F32),
            pltpu.VMEM((2, 8, 128), I32),
            pltpu.SemaphoreType.DMA((5,)),
            pltpu.SemaphoreType.DMA((11,)),
            pltpu.SemaphoreType.DMA((8,)),
        ],
        compiler_params=pltpu.CompilerParams(
            vmem_limit_bytes=127 * 1024 * 1024,
            flags={"XLA_TPU_RESCHEDULE_DMA_DONES": True},
            disable_bounds_checks=True,
            disable_semaphore_checks=True,
        ),
    )(tiles.reshape(144, 8, PAIRS, 16, 128), w, b)
    return out.reshape(16, 72, 32, 8, 128).transpose(0, 2, 4, 1, 3).reshape(x.shape)
```
